```python
import jax
import jax.numpy as jnp

def _softmax(x, axis=-1):
    return jax.nn.softmax(x, axis=axis)
def _gelu(x):
    return jax.nn.gelu(x, approximate=True)
def _silu(x):
    return jax.nn.silu(x)
def _sigmoid(x):
    return jax.nn.sigmoid(x)
def _layernorm(x, axis=-1, eps=1e-5):
    m = jnp.mean(x, axis=axis, keepdims=True)
    v = jnp.var(x, axis=axis, keepdims=True)
    return (x - m) / jnp.sqrt(v + eps)
def _scatter_add(tgt, idx, src, axis=0):
    return tgt.at[idx].add(src)
def _segment_sum(src, seg, n):
    return jax.ops.segment_sum(src, seg, n)
class _Rng:
    def __init__(self, key):
        self._k = key
    def _next(self):
        self._k, sub = jax.random.split(self._k)
        return sub
    def normal(self, shape):
        return jax.random.normal(self._next(), shape, dtype=jnp.bfloat16)
    def randint(self, lo, hi, shape):
        return jax.random.randint(self._next(), shape, lo, hi, dtype=jnp.int32)
    def uniform(self, shape, lo=0.0, hi=1.0):
        return jax.random.uniform(self._next(), shape, jnp.bfloat16, lo, hi)
    def permutation(self, n):
        return jax.random.permutation(self._next(), n)


kernel_name = 'parallel_sum__sliding_local_dilated__mixer_channel_mlp__prompt'

def _fwd_setup_inputs():
    _rng = _Rng(jax.random.key(int.from_bytes(__import__("os").urandom(4), "little")))
    _w = (lambda a: (lambda t: t.astype(jnp.bfloat16) if jnp.issubdtype(t.dtype, jnp.floating) else t)(jnp.asarray(a)))
    def _A_setup():
        B, S, D = 1, 2048, 576
        return {
            "x": _w((lambda *s: _rng.normal(s) * 0.05)(B, S, D)),
            "wqkv": _w((lambda *s: _rng.normal(s) * 0.05)(D, 3 * D)),
            "wo": _w((lambda *s: _rng.normal(s) * 0.05)(D, D)),
        }
    _A_in = _A_setup()

    def _B_setup():
        B, S, D, F = 1, 2048, 576, 4608
        return {
            "x": _w((lambda *s: _rng.normal(s) * 0.05)(B, S, D)),
            "w1": _w((lambda *s: _rng.normal(s) * 0.05)(D, F) * (D ** -0.5)),
            "b1": _w((lambda *s: _rng.normal(s) * 0.05)(F)),
            "w2": _w((lambda *s: _rng.normal(s) * 0.05)(F, D) * (F ** -0.5)),
            "b2": _w((lambda *s: _rng.normal(s) * 0.05)(D)),
        }
    _B_in = _B_setup()

    return {
        "A_x": _A_in["x"],
        "A_wqkv": _A_in["wqkv"],
        "A_wo": _A_in["wo"],
        "B_x": _B_in["x"],
        "B_w1": _B_in["w1"],
        "B_b1": _B_in["b1"],
        "B_w2": _B_in["w2"],
        "B_b2": _B_in["b2"],
    }

def _fwd_reference(A_x, A_wqkv, A_wo, B_x, B_w1, B_b1, B_w2, B_b2):
    def _A_ref(x, wqkv, wo):
        B, S, D = x.shape
        H = 32; Dh = D // H
        W, dil = 8, 2
        qkv = (lambda x, *d: x.transpose(*d))((x @ wqkv).reshape(B, S, 3, H, Dh), 2, 0, 3, 1, 4)
        q, k, v = qkv[0], qkv[1], qkv[2]
        scale = Dh ** -0.5
        pos = jnp.arange(S)
        off = jnp.arange(W) * dil
        idx = pos[:, None] - off[None, :]
        mask = idx >= 0
        idx_c = jnp.where(mask, idx, 0).reshape(-1)
        kg = k[:, :, idx_c, :].reshape(B, H, S, W, Dh)
        vg = v[:, :, idx_c, :].reshape(B, H, S, W, Dh)
        logits = jnp.einsum("bhsd,bhswd->bhsw", q, kg) * scale
        logits = jnp.where(mask[None, None, :, :], logits, -1e9)
        attn = _softmax(logits, axis=-1)
        o = jnp.einsum("bhsw,bhswd->bhsd", attn, vg)
        return (lambda x, *d: x.transpose(*d))(o, 0, 2, 1, 3).reshape(B, S, D) @ wo

    def _B_ref(x, w1, b1, w2, b2):
        y = _layernorm(x, axis=-1)
        h = _gelu(jnp.einsum("bsd,df->bsf", y, w1) + b1)
        return jnp.einsum("bsf,fd->bsd", h, w2) + b2

    x = A_x
    xn = _layernorm(x, axis=-1)
    return x + _A_ref(xn, A_wqkv, A_wo) + _B_ref(xn, B_w1, B_b1, B_w2, B_b2)


def setup_inputs():
    _inp = _fwd_setup_inputs()
    _gk = jax.random.fold_in(jax.random.key(int.from_bytes(__import__("os").urandom(4), "little")), 2**31 - 1)
    _shapes = [[1, 2048, 576]]
    _dtypes = ['bfloat16']
    _gks = jax.random.split(_gk, len(_shapes))
    _gs = [jax.random.normal(k, s, dtype=jnp.dtype(d)) * 0.05 for k, s, d in zip(_gks, _shapes, _dtypes)]
    _inp["grad_out"] = _gs[0]
    return _inp

def reference(A_x, A_wqkv, A_wo, B_w1, B_b1, B_w2, B_b2, B_x, grad_out):
    _const = dict(B_x=B_x)
    def _f(*_d):
        return _fwd_reference(**{'A_x': _d[0], 'A_wqkv': _d[1], 'A_wo': _d[2], 'B_w1': _d[3], 'B_b1': _d[4], 'B_w2': _d[5], 'B_b2': _d[6], **_const})
    _out, _vjp = jax.vjp(_f, A_x, A_wqkv, A_wo, B_w1, B_b1, B_w2, B_b2)
    _grads = _vjp(grad_out)
    _out0 = jnp.asarray(_out)
    return (_out0, *[jnp.asarray(_g) for _g in _grads])
```

```python
import functools
import itertools
import math

import jax
import jax.numpy as jnp
from jax import lax
from jax.experimental import pallas as pl
from jax.experimental.pallas import tpu as pltpu

F32 = jnp.float32
BF16 = jnp.bfloat16
U32 = jnp.uint32

S, D, F = 2048, 576, 4608
H, DH, WIN, DIL = 32, 18, 8, 2
EPS = 1e-5
LANES = 128
HG_ROWS = 8 * DH
N_HG = H // 8
N_TILES = S // LANES

FC = 512
NB = 4
DM = 512
DR = D - DM
DB, SB, FB = DM // NB, S // NB, FC // NB
NJ = SB // LANES
NC = F // FC
N_STEPS = NC * NJ
HEAD_COLS = 3 * LANES
N_DT = DM // LANES + 1
ORDER = (0, 1, 2, 3, 4, 5, 6)

NN = (((1,), (0,)), ((), ()))
NT = (((1,), (1,)), ((), ()))

ALPHA = ({(0, 0): 1, (1, 1): 1}, {(1, 0): 1, (1, 1): 1}, {(0, 0): 1}, {(1, 1): 1},
         {(0, 0): 1, (0, 1): 1}, {(1, 0): 1, (0, 0): -1}, {(0, 1): 1, (1, 1): -1})
BETA = ({(0, 0): 1, (1, 1): 1}, {(0, 0): 1}, {(0, 1): 1, (1, 1): -1}, {(1, 0): 1, (0, 0): -1},
        {(1, 1): 1}, {(0, 0): 1, (0, 1): 1}, {(1, 0): 1, (1, 1): 1})
GAMMA = ({(0, 0): 1, (1, 1): 1}, {(1, 0): 1, (1, 1): -1}, {(0, 1): 1, (1, 1): 1},
         {(0, 0): 1, (1, 0): 1}, {(0, 1): 1, (0, 0): -1}, {(1, 1): 1}, {(0, 0): 1})
REM_PRODUCTS = (0, 1, 2, 5)


QUADS = ((0, 0), (0, 1), (1, 0), (1, 1))
PRODUCTS = [(r1, r2) for r1 in range(7) for r2 in range(7)]
BIG = [r for r in PRODUCTS if r[0] in REM_PRODUCTS and r[1] in REM_PRODUCTS]
SMALL = [r for r in PRODUCTS if r not in BIG]


def _signed_sum(terms):
    terms = [(c, v) for c, v in terms if v is not None]
    if not terms:
        return None
    terms.sort(key=lambda t: -t[0])
    c0, acc = terms[0]
    if c0 < 0:
        acc = -acc
    for c, v in terms[1:]:
        acc = acc + v if c > 0 else acc - v
    return acc


def _expand(table, blocks, keep=range(7)):
    return {r: _signed_sum([(c, blocks.get(key)) for key, c in table[r].items()]) for r in keep}


def _contract(table, products):
    terms = {}
    for r, v in products.items():
        for key, c in table[r].items():
            terms.setdefault(key, []).append((c, v))
    return {key: _signed_sum(t) for key, t in terms.items()}


def _expand_inner(table, load, r1, keep=range(7)):
    blocks = {}
    for i, j in QUADS:
        blocks[(i, j)] = _signed_sum([(c, load(2 * bi + i, 2 * bj + j)) for (bi, bj), c in table[r1].items()])
    return _expand(table, blocks, keep)


def _merge(*streams, lead=0.0):
    order = []
    for k, stream in enumerate(streams):
        order += [((i + 0.5) / len(stream) * (1.0 - lead if k else 1.0), -k, i) for i in range(len(stream))]
    return [streams[-k][i] for _, k, i in sorted(order)]


def _interleave(*streams):
    for thunk in _merge(*streams):
        thunk()


def _dot(a, b, dims):
    return lax.dot_general(a, b, dims, preferred_element_type=F32)


def _pack(lo, hi):
    return pltpu.bitcast(pltpu.pack_elementwise([lo, hi], packed_dtype=BF16), U32)


def _unpack(words):
    return [pltpu.unpack_elementwise(words, index=i, packed_dtype=BF16, unpacked_dtype=F32) for i in range(2)]


def _bf16(words):
    return pltpu.bitcast(words, BF16)


def _row_pairs(tile):
    return _Pair(*_unpack(pltpu.bitcast(tile, U32)))


class _Pair:
    def __init__(self, lo, hi):
        self.lo, self.hi = lo, hi

    def __add__(self, other):
        return _Pair(self.lo + other.lo, self.hi + other.hi)

    def __sub__(self, other):
        return _Pair(self.lo - other.lo, self.hi - other.hi)

    def __neg__(self):
        return _Pair(-self.lo, -self.hi)

    def words(self):
        return _pack(self.lo, self.hi)


def _colsum(v):
    return jnp.sum(v, axis=0, keepdims=True)


def _layernorm_t(v):
    cen = v - _colsum(v) * (1.0 / D)
    rstd = lax.rsqrt(_colsum(cen * cen) * (1.0 / D) + EPS)
    return cen * rstd, rstd


def _layernorm_t_bwd(dn, n, rstd):
    return rstd * (dn - _colsum(dn) * (1.0 / D) - n * (_colsum(dn * n) * (1.0 / D)))


def _gelu_and_grad(p):
    c = math.sqrt(2.0 / math.pi)
    a = 0.044715
    p2 = p * p
    t = jnp.tanh(p * (c + (c * a) * p2))
    cdf = 0.5 + 0.5 * t
    h = p * cdf
    return h, cdf + h * (1.0 - cdf) * (2.0 * c + (6.0 * c * a) * p2)


class _Comb:
    def __init__(self, big, small, *index):
        self.big, self.small, self.index = big, small, index

    def at(self, r):
        ref, slot = (self.big, BIG.index(r)) if r in BIG else (self.small, SMALL.index(r))
        return ref.at[(*self.index, slot)]


def _tile(i, size=LANES):
    return pl.ds(i * size if isinstance(i, int) else pl.multiple_of(i * size, size), size)


def _each(fn, *ranges):
    return [functools.partial(fn, *args) for args in itertools.product(*ranges)]


def _kernel(x_hbm, wqkv_hbm, wo_hbm, w1_hbm, b1_ref, w2_hbm, b2_ref, g_hbm,
            out_hbm, dx_hbm, dwqkv_hbm, dwo_hbm, dw1_hbm, db1_ref, dw2_hbm, db2_ref,
            x_v, g_v, xn_v, wqkv_v, wo_v, dqkv_v, o_v, dwo_v, mlp_out, acco_m, acco_r, accy_m, accy_r,
            in_sem, w_sem, dw_sem, out_sem, zero_ref):
    acc_t1 = ((accy_m, accy_r), (acco_m, acco_r))
    dwo_copy = pltpu.make_async_copy(dwo_v, dwo_hbm, out_sem.at[0])

    def gather(which, j, dst):
        main_ref, rem_ref = acc_t1[which]
        for rt in range(0, DB, 8):
            for n, (ki, si) in enumerate(QUADS):
                blocks = _contract(BETA, {r1: main_ref[j, 4 * r1 + n, rt:rt + 8, :] for r1 in range(7)})
                for (ko, so), v in blocks.items():
                    dst[j, 2 * so + si, pl.ds((2 * ko + ki) * DB + rt, 8), :] = v
        for rt in range(0, DR, 8):
            for si in range(2):
                blocks = _contract(BETA, {r1: rem_ref[j, 2 * n + si, rt:rt + 8, :]
                                          for n, r1 in enumerate(REM_PRODUCTS)})
                for so in range(2):
                    dst[j, 2 * so + si, pl.ds(DM + rt, 8), :] = blocks[(0, so)]

    def main(yc_b, yc_s, gc_b, gc_s, w1c_b, w1c_s, w2c_b, w2c_s, w1t_b, w1t_s, w2t_b, w2t_s,
             pre_v, hid_v, hcomb, dcomb, dw1_m, dw1_r, dw2_m, dw2_r, wraw, wraw_t, dw_stage,
             qkv_v, db1_acc, db1_v, att_out, att_carry, dwqkv_v, head_v, b1_v):
        t1comb = ((yc_b, yc_s), (gc_b, gc_s))
        wcomb = ((w1c_b, w1c_s), (w2c_b, w2c_s))
        wcomb_t = ((w1t_b, w1t_s), (w2t_b, w2t_s))
        acc_t2 = ((dw1_m, dw1_r), (dw2_m, dw2_r))
        t3comb = (dcomb, hcomb)

        zero_ref[0] = 0
        att_carry[...] = jnp.zeros(att_carry.shape, F32)
        latest, zero = [att_carry[0, 0, 0, 0]], [zero_ref[0]]

        def restart():
            latest[0], zero[0] = att_carry[0, 0, 0, 0], zero_ref[0]

        def matmul(a, b, dims):
            res = _dot(a, b, dims)
            latest[0] = res[0:8, 0:LANES]
            return res

        def mark(value, ref, row, *index):
            rows = 16 if ref.dtype == BF16 else 8
            spot = (*index, pl.ds(pl.multiple_of(zero[0] + row, rows), rows), pl.ds(0, LANES))
            if ref.dtype == BF16:
                ref[spot] = jnp.concatenate([value, value], axis=0).astype(BF16)
            else:
                ref[spot] = value if value.dtype == ref.dtype else pltpu.bitcast(value, ref.dtype)

        def paced(every, thunks, *corners):
            def run(i, thunk):
                if i % every == 0:
                    for corner in corners:
                        mark(latest[0], *corner)
                return thunk()
            return [functools.partial(run, i, thunk) for i, thunk in enumerate(thunks)] if every else thunks

        def overlap(products, operand, lead, *streams):
            lags = {thunk: lag for thunks, lag in streams for thunk in thunks}
            pending, count = [], 0
            for thunk in _merge(products, *(thunks for thunks, _ in streams), lead=lead):
                if thunk in lags:
                    place = thunk()
                    if place is not None and lags[thunk] is not None:
                        pending.append((count + lags[thunk], place))
                    continue
                for _, (ref, *index) in (p for p in pending if p[0] == count):
                    rows = 16 if ref.dtype == BF16 else 8
                    seen = ref[(*index, pl.ds(pl.multiple_of(zero[0], rows), rows), pl.ds(0, LANES))]
                    mark(seen.astype(F32)[0:8] if ref.dtype == BF16 else seen, *operand)
                count += 1
                thunk()

        def w_copy(c, which):
            return pltpu.make_async_copy((w1_hbm, w2_hbm)[which].at[:, _tile(c, FC)], wraw.at[c, which, 0:D],
                                         w_sem.at[c, which])

        def dw_copy(c, which):
            return pltpu.make_async_copy(dw_stage.at[c % 2, which], (dw1_hbm, dw2_hbm)[which].at[:, _tile(c, FC)],
                                         dw_sem.at[c % 2, which])

        def weight_rows(c, quarter):
            raw = wraw.at[jnp.minimum(c, NC - 1)]

            def main_rows(which, part, r1):
                def load(fb, k):
                    return _row_pairs(raw[which, _tile(k * (DB // 16) + 2 * quarter + part, 16), _tile(fb)])
                for r2, v in _expand_inner(ALPHA, load, r1).items():
                    _Comb(*wcomb[which], c % 2).at((r1, r2))[_tile(2 * quarter + part, 8), :] = v.words()
                if r1 == 6:
                    return wcomb[which][1], 0, 0

            def rem_rows(which, r1):
                def load(fb, k):
                    return None if k else _row_pairs(raw[which, _tile(DM // 16 + quarter, 16), _tile(fb)])
                for r2, v in _expand_inner(ALPHA, load, r1, REM_PRODUCTS).items():
                    _Comb(*wcomb[which], c % 2).at((r1, r2))[_tile(DB // 16 + quarter, 8), :] = v.words()
                if r1 == REM_PRODUCTS[-1]:
                    return wcomb[which][0], 0, 0
            return _each(main_rows, range(2), range(2), range(7)) + _each(rem_rows, range(2), REM_PRODUCTS)

        def weight_flip(c, ft):
            chunk = jnp.minimum(c, NC - 1)

            def one(which, dt):
                if dt < NB:
                    tile = wraw[chunk, which, _tile(dt), _tile(ft)].astype(F32)
                else:
                    pad = jnp.zeros((LANES - DR, LANES), F32)
                    if which == 0:
                        first = lax.broadcasted_iota(jnp.int32, pad.shape, 0) == 0
                        pad = jnp.where(first, b1_v[chunk * NB + ft], pad)
                    tile = jnp.concatenate([wraw[chunk, which, DM:D, _tile(ft)].astype(F32), pad], axis=0)
                wraw_t[c % 2, which, dt, _tile(ft), :] = tile.T
                return wraw_t, 0, 0, 0
            return _each(one, range(2), range(N_DT))

        def weight_cols(c, quarter):
            def one(which, parity, r1):
                def load(fb, dt):
                    rows = wraw_t.at[c % 2, which, dt, _tile(fb * (FB // 32) + quarter, 32)]
                    return _Pair(rows[pl.ds(parity, 8, stride=4), :], rows[pl.ds(parity + 2, 8, stride=4), :])
                comb = _Comb(*wcomb_t[which], c % 2)
                rows = _tile(2 * quarter + parity, 8)
                for r2, v in _expand_inner(ALPHA, load, r1).items():
                    comb.at((r1, r2))[rows, 0:DB] = v.words()
                if r1 in REM_PRODUCTS:
                    for r2, v in _expand_inner(ALPHA, lambda fb, k: None if k else load(fb, NB), r1,
                                               REM_PRODUCTS).items():
                        comb.at((r1, r2))[rows, DB:] = v.words()
                if r1 == 6:
                    return wcomb_t[which][1], 0, 0
            return paced(7, _each(one, range(2), range(2), range(7)), (wraw_t, FC, 0, 0, 0))

        def up_products(t):
            res = {}

            def one(r1, which, r2):
                lhs, rhs = _Comb(*wcomb_t[which], t // NJ % 2), _Comb(*t1comb[which], t % NJ)
                res[r2] = matmul(_bf16(lhs.at((r1, r2))[...]), _bf16(rhs.at((r1, r2))[...]), NN)
                if r2 == ORDER[-1]:
                    blocks = _contract(GAMMA, res)
                    for n, key in enumerate(QUADS):
                        pre_v[which, 4 * r1 + n, 0:FB] = blocks[key]
            return _each(one, range(7), range(2), ORDER)

        def activation(t):
            total = {}

            def one(rt, n):
                rows = pl.ds(rt, 8)
                fi, si = QUADS[n]
                pre, dh = (_contract(GAMMA, {r1: pre_v[which, 4 * r1 + n, rows, :] for r1 in range(7)})
                           for which in range(2))
                dpre = {}
                for fo, so in QUADS:
                    hid, slope = _gelu_and_grad(pre[(fo, so)])
                    dpre[(fo, so)] = dh[(fo, so)] * slope
                    slot = (2 * fo + fi) * NB + 2 * so + si
                    hid_v[0, slot, rows, :] = dpre[(fo, so)]
                    hid_v[1, slot, rows, :] = hid
                for fo in range(2):
                    part = dpre[(fo, 0)] + dpre[(fo, 1)]
                    if si == 0:
                        total[fo] = part
                        continue
                    brows = pl.ds((2 * fo + fi) * FB + rt // 32 * 32 + rt % 16 * 2 + rt % 32 // 16, 8, stride=2)
                    part = part + total[fo]
                    if not isinstance(t, int):
                        part = part + jnp.where(t % NJ == 0, 0.0, db1_acc[brows, :])
                    db1_acc[brows, :] = part
                if n == 3:
                    return hid_v, 0, 0

            return paced(2, _each(one, range(0, FB, 8), range(4)), (pre_v, 0, 0, 28))

        def bias_grad(t):
            db1_v[t // NJ] = _colsum(db1_acc[...].T)

        def spread():
            def one(rt, which, r1):
                low = rt // 32 * 32 + rt % 32 // 2

                def load(fb, sb):
                    return _Pair(hid_v[which, fb * NB + sb, pl.ds(low, 8), :],
                                 hid_v[which, fb * NB + sb, pl.ds(low + 16, 8), :])
                for r2, v in _expand_inner(GAMMA, load, r1).items():
                    t3comb[which][7 * r1 + r2, pl.ds(rt // 2, 8), :] = v.words()

            def rows(r1, which):
                for rt in range(0, FB, 16):
                    one(rt, which, r1)
                return t3comb[which], 0
            return paced(1, _each(rows, range(7), range(2)), (hid_v, 0, 0, NB * NB))

        def accumulate(table, res, main_ref, rem_ref, r1, rem_keys, fresh):
            def add(ref, slots, blocks):
                rows = blocks[0].shape[0]
                old = [ref[slot, 0:rows] for slot in slots]
                for slot, prev, v in zip(slots, old, blocks):
                    ref[slot, 0:rows] = jnp.where(fresh, v, prev + v)
            blocks = _contract(table, {r2: v[0:DB] for r2, v in res.items()})
            add(main_ref, [4 * r1 + n for n in range(4)], [blocks[key] for key in QUADS])
            if r1 in REM_PRODUCTS:
                blocks = _contract(table, {r2: res[r2][DB:] for r2 in REM_PRODUCTS})
                add(rem_ref, [2 * REM_PRODUCTS.index(r1) + n for n in range(2)], [blocks[key] for key in rem_keys])

        def down_products(t):
            res = {}

            def one(r1, which, r2):
                lhs = _Comb(*wcomb[which], t // NJ % 2)
                res[r2] = matmul(_bf16(lhs.at((r1, r2))[...]), _bf16(t3comb[which][7 * r1 + r2, 0:FB // 2]), NN)
                if r2 == ORDER[-1]:
                    accumulate(BETA, res, *(ref.at[t % NJ] for ref in acc_t1[which]), r1, ((0, 0), (0, 1)),
                               fresh=t < NJ)
            return _each(one, range(7), range(2), ORDER)

        def grad_products(t):
            res = {}

            def one(r1, which, r2):
                lhs = _Comb(*t1comb[which], t % NJ).at((r1, r2))
                res[r2] = matmul(_bf16(lhs[0:(DB + DR if (r1, r2) in BIG else DB) // 2, :]),
                                 _bf16(t3comb[which][zero[0] + 7 * r1 + r2, 0:FB // 2]), NT)
                if r2 == ORDER[-1]:
                    accumulate(ALPHA, res, *(ref.at[t // NJ % 2] for ref in acc_t2[which]), r1,
                               ((0, 0), (1, 0)), fresh=t % NJ == 0)
            return _each(one, range(7), range(2), ORDER)

        def grad_finish(c, quarter):
            def main_rows(which, part, n):
                fi, ki = QUADS[n]
                src = acc_t2[which][0].at[c % 2]
                blocks = _contract(ALPHA, {r1: src[4 * r1 + n, _tile(2 * quarter + part, 16), :] for r1 in range(7)})
                for (fo, ko), v in blocks.items():
                    dw_stage[c % 2, which, _tile((2 * ko + ki) * (DB // 16) + 2 * quarter + part, 16),
                             _tile(2 * fo + fi)] = v.astype(BF16)
                if n == 3:
                    return dw_stage, 0, 0

            def rem_rows(which, fi):
                src = acc_t2[which][1].at[c % 2]
                blocks = _contract(ALPHA, {r1: src[2 * n + fi, _tile(quarter, 16), :]
                                           for n, r1 in enumerate(REM_PRODUCTS)})
                for fo in range(2):
                    dw_stage[c % 2, which, _tile(DM // 16 + quarter, 16), _tile(2 * fo + fi)] = (
                        blocks[(fo, 0)].astype(BF16))
            return _each(main_rows, range(2), range(2), range(4)) + _each(rem_rows, range(2), range(2))

        def attention(tile, groups):
            before, after = jnp.maximum(tile - 1, 0), jnp.minimum(tile + 1, N_TILES - 1)
            lane = lax.broadcasted_iota(jnp.int32, (8, LANES), 1)
            scale = DH ** -0.5
            q, k, v, do = ((qkv_v, n * D) for n in range(4))
            state = {}

            def words(base, sub, i):
                return _tile(base // 16 + groups[sub] * (HG_ROWS // 16) + i, 8)

            def head_rows(src, sub, at):
                return [src[0][words(src[1], sub, i), _tile(at)] for i in range(DH // 2)]

            def back(cur, prev, w):
                if w == 0:
                    return cur
                return pltpu.roll(jnp.where(lane < LANES - DIL * w, cur, prev), DIL * w, 1)

            def ahead(cur, nxt, w):
                if w == 0:
                    return cur
                return pltpu.roll(jnp.where(lane >= DIL * w, cur, nxt), LANES - DIL * w, 1)

            def scores(sub, src, oth, name):
                acc = [None] * WIN
                for a, cur, prev in zip(head_rows(src, sub, tile), head_rows(oth, sub, tile),
                                        head_rows(oth, sub, before)):
                    a0, a1 = _unpack(a)
                    for w in range(WIN):
                        b0, b1 = _unpack(back(cur, prev, w))
                        term = a0 * b0 + a1 * b1
                        acc[w] = term if acc[w] is None else acc[w] + term
                state[name] = acc

            def softmax(sub):
                pos = lane + tile * LANES
                logit = [jnp.where(pos >= DIL * w, state["qk"][w] * scale, -1e9) for w in range(WIN)]
                top = functools.reduce(jnp.maximum, logit)
                e = [jnp.exp(val - top) for val in logit]
                inv = 1.0 / functools.reduce(lambda a, b: a + b, e)
                attn = [val * inv for val in e]
                mean = functools.reduce(lambda a, b: a + b, [a * b for a, b in zip(attn, state["dov"])])
                dlogit = [jnp.where(pos >= DIL * w, attn[w] * (state["dov"][w] - mean) * scale, 0.0)
                          for w in range(WIN)]
                for n, (name, vals) in enumerate((("attn", attn), ("dlogit", dlogit))):
                    nxt = [jnp.where(pos < S - LANES, att_carry[(tile + 1) % 2, groups[sub], n, w], 0.0)
                           for w in range(WIN)]
                    state[name] = vals
                    state[name + "_t"] = [ahead(vals[w], nxt[w], w) for w in range(WIN)]
                for n, vals in enumerate((attn, dlogit)):
                    for w in range(WIN):
                        att_carry[tile % 2, groups[sub], n, w] = vals[w]
                return att_carry, 0, 0, 0, 0

            def mix(sub, weights, src, shift, slot, dst, base):
                other = before if shift is back else after
                for i, (cur, oth) in enumerate(zip(head_rows(src, sub, tile), head_rows(src, sub, other))):
                    shifted = [_unpack(shift(cur, oth, w)) for w in range(WIN)]
                    for n in range(2):
                        terms = [state[weights][w] * shifted[w][n] for w in range(WIN)]
                        att_out[4 * sub + slot, pl.ds(2 * i + n, 8, stride=DH), :] = functools.reduce(
                            lambda a, b: a + b, terms)
                for i in range(HG_ROWS // 16):
                    dst[words(base, sub, i), _tile(tile)] = _pack(
                        att_out[4 * sub + slot, pl.ds(16 * i, 8, stride=2), :],
                        att_out[4 * sub + slot, pl.ds(16 * i + 1, 8, stride=2), :])
                return (dst,)

            thunks = []
            for sub in range(len(groups)):
                thunks += [functools.partial(scores, sub, q, k, "qk"), functools.partial(scores, sub, do, v, "dov"),
                           functools.partial(softmax, sub),
                           functools.partial(mix, sub, "attn", v, back, 0, o_v, 0),
                           functools.partial(mix, sub, "dlogit", k, back, 1, dqkv_v, 0),
                           functools.partial(mix, sub, "dlogit_t", q, ahead, 2, dqkv_v, D),
                           functools.partial(mix, sub, "attn_t", do, ahead, 3, dqkv_v, 2 * D)]
            return thunks

        quarter_cols = S // 4
        x_copies = [pltpu.make_async_copy(x_hbm.at[0, :, _tile(i, quarter_cols)],
                                          x_v.at[0:D, _tile(i, quarter_cols)], in_sem.at[i]) for i in range(4)]
        wqkv_copy = pltpu.make_async_copy(wqkv_hbm, wqkv_v, in_sem.at[4])
        g_copy = pltpu.make_async_copy(g_hbm.at[0], g_v.at[0:D], in_sem.at[5])
        wo_copy = pltpu.make_async_copy(wo_hbm, wo_v, in_sem.at[6])
        head_copy = pltpu.make_async_copy(wqkv_hbm.at[:, pl.ds(0, HEAD_COLS)], head_v, in_sem.at[7])

        def norm_tile(t):
            x = _row_pairs(x_v[0:D, _tile(t)])
            xn, _ = _layernorm_t(jnp.concatenate([x.lo, x.hi], axis=0))
            xn_v[:, _tile(t)] = _pack(xn[:D // 2], xn[D // 2:])
            y, _ = _layernorm_t(xn)
            for p in range(2):
                for n, r0 in enumerate(range(0, D // 2, LANES)):
                    rows = min(LANES, D // 2 - r0)
                    accy_m[t % NJ, 6 * (t // NJ) + 3 * p + n, 0:rows, :] = y[p * (D // 2) + r0:p * (D // 2) + r0 + rows]
            return accy_m, 0, 0

        band = 2 * HG_ROWS

        def stage_wqkv(i):
            first = i * band // LANES
            for n in range(first, pl.cdiv((i + 1) * band, LANES)):
                width = min(LANES, 3 * D - n * LANES)
                tile = (wqkv_v if i else head_v)[:, n * LANES:n * LANES + width].astype(F32)
                if width < LANES:
                    tile = jnp.concatenate([tile, jnp.zeros((D, LANES - width), F32)], axis=1)
                tile = jnp.concatenate([tile, jnp.zeros((N_DT * LANES - D, LANES), F32)], axis=0)
                for dt in range(N_DT):
                    wraw_t[i % 2, 0, dt, _tile(n - first), :] = tile[dt * LANES:(dt + 1) * LANES].T
            return i * band - first * LANES

        def stage_wo(i):
            for dt in range(N_DT):
                width = min(LANES, D - dt * LANES)
                tile = wo_v[(i - 6) * band:(i - 5) * band, dt * LANES:dt * LANES + width].astype(F32)
                if width < LANES:
                    tile = jnp.concatenate([tile, jnp.zeros((band, LANES - width), F32)], axis=1)
                wraw_t[i % 2, 0, dt, 0:band, :] = tile
            return 0

        def gather_heads(i, stage):
            base = stage(i)
            for d in range(DH):
                for dt in range(N_DT):
                    words = _pack(wraw_t[i % 2, 0, dt, pl.ds(base + d, 8, stride=2 * DH), :],
                                  wraw_t[i % 2, 0, dt, pl.ds(base + DH + d, 8, stride=2 * DH), :])
                    acco_m[i // 2, 2 * (i % 2 * N_DT + dt) + d // 9, pl.ds(d % 9 * 8, 8), :] = pltpu.bitcast(words, F32)

        def project(t, i, operands):
            lhs = jnp.concatenate(
                [jnp.concatenate([acco_m[i // 2, 2 * (i % 2 * N_DT + dt) + part, 0:HG_ROWS // 2, :]
                                  for part in range(2)], axis=0) for dt in range(N_DT)], axis=1)
            res = matmul(_bf16(pltpu.bitcast(lhs, U32))[:, 0:D], operands[i // 6], NN)
            for sub in range(2):
                for d in range(0, DH, 2):
                    lo = 16 * d + 8 * sub
                    qkv_v[pl.ds((2 * i + sub) * (HG_ROWS // 2) + 4 * d, 8), _tile(t)] = _pack(
                        res[lo:lo + 8], res[lo + 16:lo + 24])

        def projections(t):
            return _each(project, [t], range(8), [(_bf16(xn_v[:, _tile(t)]), g_v[0:D, _tile(t)])])

        def t1_combos(which, load):
            def main_rows(j, rt):
                for r1 in range(7):
                    for r2, v in _expand_inner(BETA, lambda k, sb: load((k, rt), sb * NJ + j), r1).items():
                        _Comb(*t1comb[which], j).at((r1, r2))[_tile(rt // 16, 8), :] = v.words()
                return t1comb[which][1], 0, 0

            def rem_rows(j):
                pad = (LANES - DR) // 2
                first = (lax.broadcasted_iota(jnp.int32, (pad, LANES), 0) == 0).astype(F32)
                blank = jnp.zeros((pad, LANES), F32)
                comb = _Comb(*t1comb[which], j)
                for r1 in REM_PRODUCTS:
                    for rt in range(0, DR, 16):
                        for r2, v in _expand_inner(BETA, lambda k, sb: None if k else load((NB, rt), sb * NJ + j),
                                                   r1, REM_PRODUCTS).items():
                            comb.at((r1, r2))[pl.ds((DB + rt) // 2, 8), :] = v.words()
                    for r2, v in _expand_inner(BETA, lambda k, sb: None if k else first, r1, REM_PRODUCTS).items():
                        comb.at((r1, r2))[pl.ds((DB + DR) // 2, pad), :] = _pack(blank if which else v, blank)
                return t1comb[which][0], 0, 0
            return main_rows, rem_rows

        def load_y(r0, t):
            k, rt = r0
            rows = _tile(k % 2 * (DB // 16) + rt // 16, 8)
            return _Pair(*(accy_m[t % NJ, 6 * (t // NJ) + 3 * p + k // 2, rows, :] for p in range(2)))

        def load_g(r0, t):
            return _row_pairs(g_v[_tile(r0[0] * (DB // 16) + r0[1] // 16, 16), _tile(t)])

        def bias2_grad():
            gsum = g_v[0:D, 0:LANES].astype(F32)
            for t in range(1, N_TILES):
                gsum = gsum + g_v[0:D, _tile(t)].astype(F32)
            gsum = jnp.concatenate([gsum, jnp.zeros((N_DT * LANES - D, LANES), F32)], axis=0)
            db2_ref[...] = _colsum(gsum.T)[:, :D].reshape(D).astype(BF16)

        x_copies[3].start()
        bias = b1_ref[...].astype(F32).reshape(1, F)
        for i in range(F // LANES):
            b1_v[i] = bias[:, i * LANES:(i + 1) * LANES]
        def prologue():
            head_copy.start()
            x_copies[3].wait()
            wqkv_copy.start()
            top = N_TILES - 1
            norm_tile(top)
            norm_tile(top - 1)
            head_copy.wait()
            for cp in [g_copy, wo_copy] + x_copies[2::-1]:
                cp.start()
            (y_main, y_rem), (g_main, g_rem) = t1_combos(0, load_y), t1_combos(1, load_g)
            for i in range(6):
                if i == 1:
                    wqkv_copy.wait()
                    for cp in [w_copy(c, n) for c in range(2) for n in range(2)]:
                        cp.start()
                gather_heads(i, stage_wqkv)
                project(top, i, [_bf16(xn_v[:, _tile(top)])])
            g_copy.wait()
            wo_copy.wait()
            for i in range(6, 8):
                gather_heads(i, stage_wo)
                project(top, i, [None, g_v[0:D, _tile(top)]])
            bias2_grad()
            for rt in range(DB // 2, DB, 16):
                g_main(NJ - 1, rt)
            for cp in x_copies[:3]:
                cp.wait()
            for which in range(2):
                for c in range(2):
                    w_copy(c, which).wait()
                for c in range(2, NC):
                    w_copy(c, which).start()

            def early_step(i, carry):
                restart()
                piece = 2 * i
                overlap(projections(top - 1 - i), None, 0.25,
                        (_each(norm_tile, [jnp.maximum(top - 2 - 2 * i - n, 0) for n in range(2)]), None),
                        (_each(g_main, [piece // 4], [piece % 4 * 32 + rt for rt in range(0, 64, 16)]), None),
                        (weight_rows(0, jnp.minimum(i, NJ - 1)) + weight_flip(i // NB, i % NB), None))
                return carry

            def late_step(i, carry):
                restart()
                cols, rem = jnp.minimum(i, NB), jnp.minimum(i, NJ - 1)
                overlap(projections(top // 2 - i), None, 0.25,
                        (_each(y_main, [i // 2], [i % 2 * 64 + rt for rt in range(0, 64, 16)]), None),
                        (weight_cols(cols // NB, cols % NB), None), (_each(g_rem, [rem]) + _each(y_rem, [rem]), None))
                return carry

            lax.fori_loop(0, top // 2, early_step, 0)
            restart()
            _interleave(weight_flip(1, NB - 1))
            lax.fori_loop(0, top // 2, late_step, 0)
            restart()
            for which in range(2):
                w_copy(2, which).wait()
            _interleave(up_products(0), _each(y_main, [NJ - 1], range(DB // 2, DB, 16)))
            overlap(projections(0), None, 0.25, (activation(0) + weight_flip(2, 0), None))

        prologue()

        def step(s, carry):
            @pl.when(jnp.logical_and((s + 1) % NJ == 0, (s + 1) // NJ + 2 < NC))
            def _():
                for which in range(2):
                    w_copy((s + 1) // NJ + 2, which).wait()

            @pl.when(jnp.logical_and(s % NJ == 0, s >= 3 * NJ))
            def _():
                for which in range(2):
                    dw_copy(s // NJ - 3, which).wait()

            @pl.when(jnp.logical_and(s % NJ == 0, s >= 2 * NJ))
            def _():
                for which in range(2):
                    dw_copy(s // NJ - 2, which).start()

            restart()
            late = jnp.minimum(s, 2 * N_TILES - 1)
            att = attention(N_TILES - 1 - late % N_TILES, [late // N_TILES * 2 + n for n in range(2)])
            cut = int(len(att) * 0.5)
            nxt = s + 1
            act = activation(nxt)
            rows = weight_rows(s // NJ + 1, s % NJ)
            down, grad = down_products(s), grad_products(s)
            flips = weight_flip(nxt // NJ + 2, nxt % NJ)
            cols = weight_cols(nxt // NJ + 1, nxt % NJ)
            half, a_cut, c_cut = int(len(att) * 0.9), int(len(act) * 0.5), int(len(cols) * 0.6)
            overlap(up_products(nxt), (yc_s, 0, 0, len(SMALL)), 0.1, (spread(), 20), (rows, 24),
                    (grad_finish(s // NJ + 1, s % NJ), 28), (att[:cut], 60),
                    ([functools.partial(bias_grad, s)], None))
            overlap(grad, (yc_s, 0, 0, len(SMALL)), 0.17, (act[:a_cut], 60), (att[cut:half], 60),
                    (cols[:c_cut], 60))
            overlap(down, (w1c_s, 0, 0, len(SMALL)), 0.17, (act[a_cut:], 60), (att[half:], 60),
                    (cols[c_cut:] + flips, 60))
            return carry

        lax.fori_loop(0, N_STEPS - 1, step, 0)

        last = N_STEPS - 1
        restart()
        for which in range(2):
            dw_copy(NC - 3, which).wait()

        def dwqkv_piece(m, n):
            words = dqkv_v[pl.ds(m // 2 if isinstance(m, int) else pl.multiple_of(m // 2, LANES), n // 2), :]
            return _dot(_bf16(xn_v[...]), _bf16(words), NT).astype(BF16)

        tail = 3 * D // 256 * 256

        def dwqkv_tail():
            dwqkv_v[:, tail:] = dwqkv_piece(tail, 3 * D - tail)

        _interleave([dwqkv_tail], spread(), grad_finish(NC - 2, NJ - 1), [functools.partial(bias_grad, last)])
        for which in range(2):
            dw_copy(NC - 2, which).start()
        _interleave(down_products(last) + grad_products(last))

        def dwqkv_step(i, carry):
            dwqkv_v[:, _tile(i, 256)] = dwqkv_piece(i * 256, 256)
            _interleave(grad_finish(NC - 1, jnp.minimum(i, NJ - 1)))
            gather(1, jnp.clip(i - 2, 0, NJ - 1), mlp_out)
            return carry

        lax.fori_loop(0, tail // 256, dwqkv_step, 0)
        dwqkv_copy = pltpu.make_async_copy(dwqkv_v, dwqkv_hbm, out_sem.at[1])
        dwqkv_copy.start()
        for which in range(2):
            dw_copy(NC - 1, which).start()

        def dwo_step(i, carry):
            dwo_v[_tile(i, D // 3), :] = _dot(_bf16(o_v[_tile(i, D // 6), :]), g_v[0:D, :], NT).astype(BF16)
            return carry

        lax.fori_loop(0, 3, dwo_step, 0)
        dwo_copy.start()
        db1_ref[...] = jnp.concatenate([db1_v[c] for c in range(NC)], axis=1).reshape(F).astype(BF16)
        dwqkv_copy.wait()
        for c in range(NC - 2, NC):
            for which in range(2):
                dw_copy(c, which).wait()

    nb, ns = len(BIG), len(SMALL)
    t1 = [pltpu.VMEM((NJ, nb, (DB + LANES) // 2, LANES), U32), pltpu.VMEM((NJ, ns + 1, DB // 2, LANES), U32)]
    wc = [pltpu.VMEM((2, nb, (DB + DR) // 2, FB), U32), pltpu.VMEM((2, ns + 1, DB // 2, FB), U32)]
    wt = [pltpu.VMEM((2, nb, FB // 2, DB + LANES), U32), pltpu.VMEM((2, ns, FB // 2, DB), U32)]
    t3 = [pltpu.VMEM((2, 29, FB + 24, LANES), F32), pltpu.VMEM((2, NB * NB + 1, FB + 24, LANES), F32)] + [pltpu.VMEM((nb + ns, FB // 2, LANES), U32)] * 2
    t2 = [pltpu.VMEM((2, 28, DB, FB), F32), pltpu.VMEM((2, 8, DR, FB), F32)]
    pl.run_scoped(
        main, *t1, *t1, *wc, *wc, *wt, *wt, *t3, *t2, *t2,
        pltpu.VMEM((NC, 2, D + 16, FC), BF16), pltpu.VMEM((2, 2, N_DT, FC + 8, LANES), F32), pltpu.VMEM((2, 2, D, FC), BF16),
        pltpu.VMEM((2 * D + 8, S), U32),
        pltpu.VMEM((FC, LANES), F32), pltpu.VMEM((NC, 1, FC), F32),
        pltpu.VMEM((8, HG_ROWS, LANES), F32), pltpu.VMEM((2, N_HG, 2, WIN, 8, LANES), F32),
        pltpu.VMEM((D, 3 * D), BF16), pltpu.VMEM((D, HEAD_COLS), BF16), pltpu.VMEM((F // LANES, 1, LANES), F32))

    def epilogue(out_v, dx_v, mlp_dy, b2_v, datt0, datt1, wo_t):
        b2 = jnp.concatenate([b2_ref[...].astype(F32).reshape(1, D), jnp.zeros((1, N_DT * LANES - D), F32)], axis=1)
        b2_v[...] = jnp.broadcast_to(b2, (LANES, N_DT * LANES)).T

        wide = jnp.concatenate([wo_v[...].astype(F32), jnp.zeros((D, N_DT * LANES - D), F32)], axis=1)
        wide = jnp.concatenate([wide, jnp.zeros((N_DT * LANES - D, N_DT * LANES), F32)], axis=0)
        wo_t[...] = wide.T[0:D].astype(BF16)

        def out_step(sb, carry):
            att = _dot(wo_t[:, 0:D], _bf16(o_v[:, _tile(sb, SB)]), NN)
            for j in range(NJ):
                t = _tile(sb * NJ + j)
                out_v[:, t] = (x_v[0:D, t].astype(F32) + att[:, j * LANES:(j + 1) * LANES] + mlp_out[j, sb]
                               + b2_v[0:D, :]).astype(BF16)
            gather(0, sb, mlp_dy)
            return carry

        lax.fori_loop(0, NB, out_step, 0)
        out_copy = pltpu.make_async_copy(out_v, out_hbm.at[0], out_sem.at[2])
        out_copy.start()

        def dx_copy(sb):
            return pltpu.make_async_copy(dx_v.at[:, _tile(sb, SB)], dx_hbm.at[0, :, _tile(sb, SB)], out_sem.at[3 + sb])

        def norm_bwd(half, datt):
            for n in range(2):
                t = _tile(2 * half + n)
                xn, rstd1 = _layernorm_t(x_v[0:D, t].astype(F32))
                y, rstd2 = _layernorm_t(xn)
                dxn = datt[:, _tile(n)] + _layernorm_t_bwd(mlp_dy[half % 2 * 2 + n, half // 2], y, rstd2)
                dx_v[:, t] = (g_v[0:D, t].astype(F32) + _layernorm_t_bwd(dxn, xn, rstd1)).astype(BF16)

        def dx_step(sb, carry):
            datt0[...] = _dot(wqkv_v[...], _bf16(dqkv_v[:, _tile(2 * sb, 2 * LANES)]), NN)
            norm_bwd(jnp.abs(2 * sb - 1), datt1)
            datt1[...] = _dot(wqkv_v[...], _bf16(dqkv_v[:, _tile(2 * sb + 1, 2 * LANES)]), NN)
            norm_bwd(2 * sb, datt0)

            @pl.when(sb > 0)
            def _():
                dx_copy(sb - 1).start()
            return carry

        datt1[...] = jnp.zeros(datt1.shape, F32)
        lax.fori_loop(0, NB, dx_step, 0)
        norm_bwd(2 * NB - 1, datt1)
        dx_copy(NB - 1).start()
        dwo_copy.wait()
        out_copy.wait()
        for sb in range(NB):
            dx_copy(sb).wait()

    pl.run_scoped(epilogue, pltpu.VMEM((D, S), BF16), pltpu.VMEM((D, S), BF16),
                  pltpu.VMEM((NJ, NB, D, LANES), F32), pltpu.VMEM((N_DT * LANES, LANES), F32), *[pltpu.VMEM((D, 2 * LANES), F32)] * 2,
                  pltpu.VMEM((D, N_DT * LANES), BF16))


@jax.jit
def pallas_parallel_sum__sliding_local_dilated__mixer_channel_mlp__prompt_kernel(
    A_x: jax.Array,
    A_wqkv: jax.Array,
    A_wo: jax.Array,
    B_x: jax.Array,
    B_w1: jax.Array,
    B_b1: jax.Array,
    B_w2: jax.Array,
    B_b2: jax.Array,
    grad_out: jax.Array,
):
    del B_x
    hbm = pl.BlockSpec(memory_space=pl.ANY)
    vmem = pl.BlockSpec(memory_space=pltpu.VMEM)
    acc = [pltpu.VMEM((NJ, 28, DB, LANES), F32), pltpu.VMEM((NJ, 8, DR, LANES), F32)]
    out_t, dx_t, dwqkv, dwo, dw1, db1, dw2_t, db2 = pl.pallas_call(
        _kernel,
        in_specs=[hbm, hbm, hbm, hbm, vmem, hbm, vmem, hbm],
        out_specs=[hbm, hbm, hbm, hbm, hbm, vmem, hbm, vmem],
        out_shape=[
            jax.ShapeDtypeStruct((1, D, S), BF16), jax.ShapeDtypeStruct((1, D, S), BF16),
            jax.ShapeDtypeStruct((D, 3 * D), BF16), jax.ShapeDtypeStruct((D, D), BF16),
            jax.ShapeDtypeStruct((D, F), BF16), jax.ShapeDtypeStruct((F,), BF16),
            jax.ShapeDtypeStruct((D, F), BF16), jax.ShapeDtypeStruct((D,), BF16),
        ],
        scratch_shapes=[
            pltpu.VMEM((D + 16, S), BF16), pltpu.VMEM((D + 16, S), BF16), pltpu.VMEM((D // 2, S), U32),
            pltpu.VMEM((D, 3 * D), BF16), pltpu.VMEM((D, D), BF16),
            pltpu.VMEM((3 * D // 2, S), U32), pltpu.VMEM((D // 2, S), U32), pltpu.VMEM((D, D), BF16),
            pltpu.VMEM((NJ, NB, D, LANES), F32), *acc, *acc,
            pltpu.SemaphoreType.DMA((8,)), pltpu.SemaphoreType.DMA((NC, 2)),
            pltpu.SemaphoreType.DMA((2, 2)), pltpu.SemaphoreType.DMA((3 + NB,)), pltpu.SMEM((1,), jnp.int32),
        ],
        compiler_params=pltpu.CompilerParams(vmem_limit_bytes=127 * 1024 * 1024),
    )(jnp.swapaxes(A_x, 1, 2), A_wqkv, A_wo, B_w1, B_b1, B_w2.T, B_b2,
      jnp.swapaxes(grad_out, 1, 2))
    return (jnp.swapaxes(out_t, 1, 2), jnp.swapaxes(dx_t, 1, 2), dwqkv, dwo, dw1, db1,
            dw2_t.T, db2)
```
